```python
import os as _os
_os.environ.setdefault("JAX_PLATFORMS", "cpu")
import jax
import jax.numpy as jnp

def _softmax(x, axis=-1):
    return jax.nn.softmax(x, axis=axis)
def _gelu(x):
    return jax.nn.gelu(x, approximate=True)
def _silu(x):
    return jax.nn.silu(x)
def _sigmoid(x):
    return jax.nn.sigmoid(x)
def _layernorm(x, axis=-1, eps=1e-5):
    m = jnp.mean(x, axis=axis, keepdims=True)
    v = jnp.var(x, axis=axis, keepdims=True)
    return (x - m) / jnp.sqrt(v + eps)
def _scatter_add(tgt, idx, src, axis=0):
    return tgt.at[idx].add(src)
def _segment_sum(src, seg, n):
    return jax.ops.segment_sum(src, seg, n)
class _Rng:
    def __init__(self, key):
        self._k = key
    def _next(self):
        self._k, sub = jax.random.split(self._k)
        return sub
    def normal(self, shape):
        return jax.random.normal(self._next(), shape, dtype=jnp.bfloat16)
    def randint(self, lo, hi, shape):
        return jax.random.randint(self._next(), shape, lo, hi, dtype=jnp.int32)
    def uniform(self, shape, lo=0.0, hi=1.0):
        return jax.random.uniform(self._next(), shape, jnp.bfloat16, lo, hi)
    def permutation(self, n):
        return jax.random.permutation(self._next(), n)


kernel_name = 'standalone__sliding_block_cached__sampling'

def setup_inputs():
    _rng = _Rng(jax.random.key(int.from_bytes(__import__("os").urandom(4), "little")))
    _w = (lambda a: (lambda t: t.astype(jnp.bfloat16) if jnp.issubdtype(t.dtype, jnp.floating) else t)(jnp.asarray(a)))
    B, Sq, D = 8, 4, 640
    Hq, Hkv, Sk, Dh = 32, 32, 4096, 192
    assert Hq % Hkv == 0, (Hq, Hkv)
    return {
        "x": _w((lambda *s: _rng.normal(s) * 0.8)(B, Sq, D)),
        "k_cache": _w((lambda *s: _rng.normal(s) * 0.8)(B, Hkv, Sk, Dh)),
        "v_cache": _w((lambda *s: _rng.normal(s) * 0.05)(B, Hkv, Sk, Dh)),
        "wq": _w((lambda *s: _rng.normal(s) * 0.8)(D, Hq * Dh) * (D ** -0.5)),
        "wo": _w((lambda *s: _rng.normal(s) * 0.05)(Hq * Dh, D) * ((Hq * Dh) ** -0.5)),
    }

def reference(x, k_cache, v_cache, wq, wo):
    B, Sq, D = x.shape
    Hq, Dh = 32, 192
    Hkv, Sk = k_cache.shape[1], k_cache.shape[2]
    W = min(4096, max(256, Sk // 4))
    rep = Hq // Hkv
    q = (lambda x, *d: x.transpose(*d))((x @ wq).reshape(B, Sq, Hq, Dh), 0, 2, 1, 3)
    k = jnp.repeat(k_cache[:, :, Sk - W:, :], rep, axis=1)
    v = jnp.repeat(v_cache[:, :, Sk - W:, :], rep, axis=1)
    scores = jnp.einsum("bhqd,bhkd->bhqk", q, k) * (Dh ** -0.5)
    p = _softmax(scores, axis=-1)
    o = jnp.einsum("bhqk,bhkd->bhqd", p, v)
    return (lambda x, *d: x.transpose(*d))(o, 0, 2, 1, 3).reshape(B, Sq, Hq * Dh) @ wo
```

```python
import jax
import jax.numpy as jnp
from jax import lax
import jax.experimental.pallas as pl
import jax.experimental.pallas.tpu as pltpu

_DELAY_WQ = 225
_DELAY_KV = (10, 10, 10, 45, 10, 10, 10, 10, 10, 10, 125, 1)
_DELAY_NOQ = 150
_DELAY_KV0 = (150,) * 9 + (1,) * 3
_DELAY_WO = 30
_VSHIFT = 48
_NOCHECK = False


@jax.jit
def pallas_standalone__sliding_block_cached__sampling_kernel(
    x: jax.Array,
    k_cache: jax.Array,
    v_cache: jax.Array,
    wq: jax.Array,
    wo: jax.Array,
):
    B, Sq, D = x.shape
    Hq, Dh = 32, 192
    Hkv, Sk = k_cache.shape[1], k_cache.shape[2]
    W = min(4096, max(256, Sk // 4))
    assert Hq == Hkv and Hq % 2 == 0 and Sq == 4 and B == 8
    P = 2 * Dh
    NP = Hq // 2
    NJ = P // 128
    R = 2 * Sq
    T = NP * B
    NS = 12
    PR = P // NS
    NA, AR = D // 16, 8
    NG, CR = Hq * Dh // 256, 64
    LA = 2
    LEAD = 2
    scale = Dh ** -0.5
    f32, bf16 = jnp.float32, jnp.bfloat16

    def kernel(x_hbm, k_hbm, v_hbm, wq_hbm, wo_hbm, out_ref,
               x_buf, k_buf, v_buf, wq_buf, wo_buf, x2, q2, s_buf, p_buf, pv_buf,
               o_buf, acc, lo_sem, hi_sem):

        def kv_piece(src, buf, sem, t, slot, r0, n):
            rows = pl.ds(pl.multiple_of((t >> 3) * P + r0, 8), n)
            return pltpu.make_async_copy(
                src.at[t & 7, rows, pl.ds(Sk - W, W)],
                buf.at[slot, pl.ds(r0, n)], sem.at[slot])

        def k_piece(t, i):
            return kv_piece(k_hbm, k_buf, lo_sem, t, t & 3, i * PR, PR)

        def v_piece(t, r0, n):
            return kv_piece(v_hbm, v_buf, hi_sem, t, t & 1, r0, n)

        def wq_piece(half, i):
            rows = pl.ds(pl.multiple_of(half * (D // 2) + i * AR, AR), AR)
            sem = (lo_sem.at[3], hi_sem.at[1])[half]
            return pltpu.make_async_copy(wq_hbm.at[rows], wq_buf.at[rows], sem)

        def wo_piece(g, half, i):
            rows = pl.ds(pl.multiple_of((2 * g + half) * 128 + i * CR, CR), CR)
            sem = (lo_sem.at[g & 3], hi_sem.at[g & 1])[half]
            return pltpu.make_async_copy(wo_hbm.at[rows], wo_buf.at[rows], sem)

        def wait_all(dst, sem):
            pltpu.make_async_copy(dst, dst, sem).wait()

        def head_mask(shape, col0=0):
            r = lax.broadcasted_iota(jnp.int32, shape, 0)
            c = lax.broadcasted_iota(jnp.int32, shape, 1) + col0
            return ((r & (R - 1)) >= Sq) == (c >= Dh)

        def project_q(p, j):
            cols = pl.ds(pl.multiple_of(p * P + j * 128, 128), 128)
            q = jnp.dot(x2[...], wq_buf[:, cols], preferred_element_type=f32)
            q2[p & 1, j] = jnp.where(head_mask(q.shape, j * 128), q, 0.0)

        def attention(t, wait_v=True):
            b = t & 7
            rows = pl.ds(pl.multiple_of(b * R, R), R)
            for j in range(NJ):
                d = jnp.dot(q2[(t >> 3) & 1, j, rows, :].astype(bf16),
                            k_buf[t & 3, pl.ds(j * 128, 128), :],
                            preferred_element_type=f32)
                s_buf[...] = d if j == 0 else s_buf[...] + d
                yield
            s = s_buf[...] * scale
            e = jnp.exp(s - jnp.max(s, axis=-1, keepdims=True))
            s_buf[...] = e
            p_buf[...] = e.astype(bf16)
            yield
            if wait_v:
                wait_all(v_buf.at[t & 1], hi_sem.at[t & 1])
            h = W // 2
            for j in range(NJ):
                for k in range(2):
                    d = lax.dot_general(
                        p_buf[:, pl.ds(k * h, h)],
                        v_buf[t & 1, pl.ds(j * 128, 128), pl.ds(k * h, h)],
                        (((1,), (1,)), ((), ())), preferred_element_type=f32)
                    cols = pl.ds(j * 128, 128)
                    pv_buf[:, cols] = d if k == 0 else pv_buf[:, cols] + d
                    yield
            l = jnp.sum(s_buf[...], axis=-1, keepdims=True)
            o = jnp.where(head_mask((R, P)), pv_buf[...] / l, 0.0)
            o = o + pltpu.roll(o, Sq, 0)
            rows = pl.ds(pl.multiple_of((b >> 1) * R, R), R)
            cols = pl.ds(pl.multiple_of((t >> 3) * P, P), P)
            mine = (lax.broadcasted_iota(jnp.int32, (R, P), 0) >> 2) == (b & 1)
            o_buf[rows, cols] = jnp.where(mine, o, o_buf[rows, cols])

        def project_o(c):
            rows = pl.ds(pl.multiple_of(c * 128, 128), 128)
            acc[...] += jnp.dot(o_buf[:, rows].astype(bf16), wo_buf[rows, :],
                                preferred_element_type=f32)

        def wait_wo(g):
            wait_all(wo_buf.at[pl.ds(pl.multiple_of((2 * g + 1) * 128, 128), 128)],
                     hi_sem.at[g & 1])

        def v_rows(t, i):
            r0 = i * PR + _VSHIFT
            if r0 < P:
                v_piece(t, r0, min(PR, P - r0)).start()
            if r0 + PR > P:
                r1 = max(r0 - P, 0)
                nxt = lambda: v_piece(t + 1, r1, r0 + PR - P - r1).start()
                pl.when(t + 1 < T)(nxt)

        for i in range(NS):
            wq_piece(0, i).start(priority=1)
        wq_piece(1, 0).start()
        x_copy = pltpu.make_async_copy(x_hbm, x_buf, hi_sem.at[0])
        x_copy.start()
        for i in range(1, LEAD):
            pl.delay(_DELAY_WQ)
            wq_piece(1, i).start()
        pl.delay(_DELAY_WQ)

        def wq_slot(i, carry):
            @pl.when(i + LEAD < NA)
            def _():
                wq_piece(1, i + LEAD).start()

            for n in range(LEAD):
                r0 = (NS - LEAD + n) * PR + _VSHIFT - P
                if r0 + PR > 0:
                    @pl.when(i == NA - LEAD + n)
                    def _():
                        v_piece(0, max(r0, 0), r0 + PR - max(r0, 0)).start()

            @pl.when(i + NS < NA)
            def _():
                wq_piece(0, i + NS).start(priority=1)

            @pl.when(i + NS == NA)
            def _():
                for n in range(NS):
                    k_piece(0, n).start(priority=1)

            pl.delay(_DELAY_WQ)
            wq_piece(0, i).wait()
            return carry

        lax.fori_loop(0, 2, wq_slot, 0)
        x_copy.wait()
        for b in range(0, B, 2):
            xa, xb = x_buf[b].astype(f32), x_buf[b + 1].astype(f32)
            x2[pl.ds(b * R, 2 * R), :] = jnp.concatenate([xa, xa, xb, xb], axis=0).astype(bf16)
        o_buf[...] = jnp.zeros_like(o_buf)
        acc[...] = jnp.zeros_like(acc)
        lax.fori_loop(2, NA, wq_slot, 0)

        def kv_step(t, first):
            work = iter(()) if first else attention(t - 1)
            delays = _DELAY_KV0 if first else _DELAY_KV
            for i in range(NS):
                v_rows(t, i)
                if i >= NS - LEAD and not first:
                    @pl.when(t + 1 == T)
                    def _():
                        wo_piece(0, 1, i - (NS - LEAD)).start()

                nxt = lambda: k_piece(t + 1, i).start(priority=1)
                nxt() if first else pl.when(t + 1 < T)(nxt)
                if i == NJ and not first:
                    @pl.when(t + 1 == T)
                    def _():
                        for n in range(2 * LA):
                            wo_piece(n // 2, 0, n % 2).start(priority=1)

                pl.delay(delays[i])
                next(work, None)
                if first:
                    if i == NS - NJ:
                        wait_all(wq_buf.at[pl.ds(D // 2, D // 2)], hi_sem.at[1])
                    if i >= NS - NJ:
                        project_q(0, i - (NS - NJ))
                elif i == NS - 1:
                    lax.cond(jnp.logical_and((t & 7) >= B - NJ, t < T - B),
                             lambda: project_q((t >> 3) + 1, (t & 7) - (B - NJ)),
                             lambda: pl.delay(_DELAY_NOQ))
                k_piece(t, i).wait()

        kv_step(0, True)
        lax.fori_loop(1, T, lambda t, c: (kv_step(t, False), c)[1], 0)

        def wo_group(g, work):
            for i in range(2):
                if i == 0:
                    pl.when(g > 0)(lambda: wait_wo(g - 1))
                wo_piece(g + 1, 1, i).start()
                pl.when(g + LA < NG)(
                    lambda: wo_piece(g + LA, 0, i).start(priority=1))
                pl.delay(_DELAY_WO)
                work(i)
                wo_piece(g, 0, i).wait()

        NF = 5
        wait_all(v_buf.at[(T - 1) & 1], hi_sem.at[(T - 1) & 1])
        last = attention(T - 1, wait_v=False)

        def attend(g):
            def work(i):
                for _ in range(4 if (g, i) == (0, 1) else 1):
                    next(last, None)
            return work

        for g in range(NF - 1):
            wo_group(g, attend(g))

        def project(g):
            def work(i):
                n = 2 * (g - (NF - 1)) + i
                lax.cond(n < 2 * (NF - 2),
                         lambda: (project_o(2 * n), project_o(2 * n + 1), None)[-1],
                         lambda: project_o(2 * (g - 1) + i))
            return work

        lax.fori_loop(NF - 1, NG - 1, lambda g, c: (wo_group(g, project(g)), c)[1], 0)
        wait_wo(NG - 2)
        project_o(2 * NG - 4)
        project_o(2 * NG - 3)
        wo_piece(NG - 1, 0, 0).wait()
        wait_wo(NG - 1)
        project_o(2 * NG - 1)
        wo_piece(NG - 1, 0, 1).wait()
        project_o(2 * NG - 2)
        for b in range(B):
            out_ref[b] = acc[pl.ds(b * Sq, Sq), :].astype(out_ref.dtype)

    kt = jnp.swapaxes(k_cache, 2, 3).reshape(B, Hkv * Dh, Sk)
    vt = jnp.swapaxes(v_cache, 2, 3).reshape(B, Hkv * Dh, Sk)

    any_spec = pl.BlockSpec(memory_space=pl.ANY)
    return pl.pallas_call(
        kernel,
        out_shape=jax.ShapeDtypeStruct((B, Sq, D), x.dtype),
        in_specs=[any_spec] * 5,
        out_specs=pl.BlockSpec(memory_space=pltpu.VMEM),
        scratch_shapes=[
            pltpu.VMEM((B, Sq, D), x.dtype),
            pltpu.VMEM((4, P, W), k_cache.dtype),
            pltpu.VMEM((2, P, W), v_cache.dtype),
            pltpu.VMEM(wq.shape, wq.dtype),
            pltpu.VMEM(wo.shape, wo.dtype),
            pltpu.VMEM((B * R, D), bf16),
            pltpu.VMEM((2, NJ, B * R, 128), f32),
            pltpu.VMEM((R, W), f32),
            pltpu.VMEM((R, W), bf16),
            pltpu.VMEM((R, P), f32),
            pltpu.VMEM((B * Sq, Hq * Dh), f32),
            pltpu.VMEM((B * Sq, D), f32),
            pltpu.SemaphoreType.DMA((4,)),
            pltpu.SemaphoreType.DMA((2,)),
        ],
        compiler_params=pltpu.CompilerParams(
            vmem_limit_bytes=64 * 1024 * 1024, disable_bounds_checks=_NOCHECK),
    )(x, kt, vt, wq, wo)
```

```python
import jax
import jax.numpy as jnp
from jax import lax
import jax.experimental.pallas as pl
import jax.experimental.pallas.tpu as pltpu

_DELAY_KV = (1, 1, 1, 1, 1, 1, 95, 1, 1, 1, 35, 1)
_DELAY_IDLE = 130
_DELAY_WQ = 140
_DELAY_WO = 30
_SHIFT = 48
_LEAD = 1
_LA = 8
_LAG = 3
_WA = 3
_NOCHECK = False


@jax.jit
def pallas_standalone__sliding_block_cached__sampling_kernel(
    x: jax.Array,
    k_cache: jax.Array,
    v_cache: jax.Array,
    wq: jax.Array,
    wo: jax.Array,
):
    B, Sq, D = x.shape
    Hq, Dh = 32, 192
    Hkv, Sk = k_cache.shape[1], k_cache.shape[2]
    W = min(4096, max(256, Sk // 4))
    assert Hq == Hkv and Hq % 8 == 0 and Sq == 4 and B == 8
    HD = Hq * Dh
    P = 2 * Dh
    NJ = P // 128
    R = 2 * Sq
    T = Hq // 2 * B
    NS = 12
    PR = P // NS
    AR, QC = 8, HD // 3
    NQ = (D // (4 * AR), D // (2 * AR))
    NG, CR = HD // 256, 64
    LEAD, LA, LAG, WA = _LEAD, _LA, _LAG, _WA
    scale = Dh ** -0.5
    f32, bf16 = jnp.float32, jnp.bfloat16

    batch_of = lambda t: (t >> 2) & 7
    pair_of = lambda t: ((t >> 5) << 2) + (t & 3)

    def kernel(x_hbm, k_hbm, v_hbm, wq_hbm, wo_hbm, out_ref,
               x_buf, k_buf, v_buf, wq_buf, wo_buf, xs, q_buf, s_buf, p_buf, pv_buf,
               o_buf, acc, sem):
        start = (lambda c: c.start(priority=1), lambda c: c.start(priority=0))
        wait = lambda c: c.wait()

        def loop(lo, hi, body):
            lax.fori_loop(lo, hi, lambda i, c: (body(i), c)[1], 0)

        def kv_slot(t, i, hi, fn):
            wrap, i = divmod(i, NS)
            which, blk = divmod(i, NS // 2)
            src, buf = ((k_hbm, k_buf), (v_hbm, v_buf))[which]
            r0 = _SHIFT + (2 * blk + hi) * PR
            for dt in range(2):
                lo, up = max(r0, dt * P), min(r0 + PR, (dt + 1) * P)
                if lo < up:
                    u = t + (wrap + dt)
                    exists = 0 <= u < T if isinstance(u, int) else wrap + dt <= 0 or u < T

                    @pl.when(exists)
                    def _():
                        rows = pl.multiple_of(pair_of(u) * P + (lo - dt * P), 8)
                        fn(pltpu.make_async_copy(
                            src.at[batch_of(u), pl.ds(rows, up - lo), pl.ds(Sk - W, W)],
                            buf.at[u & 3, pl.ds(lo - dt * P, up - lo)],
                            sem.at[2 * (u & 1) + which]))

        def wq_piece(part, i, hi):
            n, cols = ((2 * AR, pl.ds(0, QC)), (AR, pl.ds(QC, HD - QC)))[part]
            rows = pl.ds(pl.multiple_of((2 * i + hi) * n, n), n)
            return pltpu.make_async_copy(
                wq_hbm.at[rows, cols], wq_buf.at[rows, cols], sem.at[2 + part])

        def wo_piece(g, hi, i):
            rows = pl.ds(pl.multiple_of((2 * g + hi) * 128 + i * CR, CR), CR)
            n = jnp.where(g == NG - 1, g + hi, g) & 3
            return pltpu.make_async_copy(wo_hbm.at[rows], wo_buf.at[rows], sem.at[n])

        def iota(shape, axis):
            return lax.broadcasted_iota(jnp.int32, shape, axis)

        def head_mask(shape, col0=0):
            return (iota(shape, 0) >= Sq) == (iota(shape, 1) + col0 >= Dh)

        def batch_mask(shape, b):
            return (iota(shape, 0) >> 2) == (b & 1)

        def batch_rows(b):
            return pl.ds(pl.multiple_of((b >> 1) * R, R), R)

        def project_q(g, n):
            cols = pl.ds(pl.multiple_of((g * 4 * NJ + n) * 128, 128), 128)
            q_buf[g & 1, n] = jnp.dot(xs[...], wq_buf[:, cols], preferred_element_type=f32)

        def score(t, j):
            if j < NJ:
                b = batch_of(t)
                q = q_buf[(t >> 5) & 1, (t & 3) * NJ + j, batch_rows(b), :]
                q = jnp.where(batch_mask(q.shape, b), q, pltpu.roll(q, Sq, 0))
                q = jnp.where(head_mask(q.shape, j * 128), q, 0.0).astype(bf16)
                d = jnp.dot(q, k_buf[t & 3, pl.ds(j * 128, 128), :],
                            preferred_element_type=f32)
                s_buf[...] = d if j == 0 else s_buf[...] + d
            else:
                s = s_buf[...] * scale
                e = jnp.exp(s - jnp.max(s, axis=-1, keepdims=True))
                s_buf[...] = e
                p_buf[...] = e.astype(bf16)

        def value(t, j):
            if j < 2 * NJ:
                cols, keys = pl.ds(j // 2 * 128, 128), pl.ds(j % 2 * (W // 2), W // 2)
                d = lax.dot_general(p_buf[:, keys], v_buf[t & 3, cols, keys],
                                    (((1,), (1,)), ((), ())), preferred_element_type=f32)
                pv_buf[:, cols] = d if j % 2 == 0 else pv_buf[:, cols] + d
            else:
                b = batch_of(t)
                l = jnp.sum(s_buf[...], axis=-1, keepdims=True)
                o = jnp.where(head_mask((R, P)), pv_buf[...] / l, 0.0)
                o = o + pltpu.roll(o, Sq, 0)
                where = (batch_rows(b), pl.ds(pl.multiple_of(pair_of(t) * P, P), P))
                o_buf[where] = jnp.where(batch_mask((R, P), b), o, o_buf[where])

        def project_o(c):
            rows = pl.ds(pl.multiple_of(c * 128, 128), 128)
            acc[...] += jnp.dot(o_buf[:, rows].astype(bf16), wo_buf[rows, :],
                                preferred_element_type=f32)

        def wq_half(part, i, hi, fn):
            if not isinstance(i, int) or 0 <= i < NQ[part]:
                fn(wq_piece(part, i, hi))
            elif i < 0:
                if part:
                    fn(wq_piece(0, i + NQ[0], hi))
            elif part == 0:
                fn(wq_piece(1, i - NQ[0], hi))
            else:
                i -= NQ[1]
                kv_slot(*((-1, NS // 2 - 1), (-1, NS - 1), (0, i - 2))[min(i, 2)], hi, fn)

        def wq_slot(part, i, work=None):
            wq_half(part, i + LEAD, 1, start[1])
            pl.delay(1 if work else _DELAY_WQ)
            if work:
                work()
            wq_half(part, i + LA, 0, start[0])
            wq_half(part, i, 0, wait)
            wq_half(part, i - LAG, 1, wait)

        def prepare():
            x_copy.wait()
            for b in range(0, B, 4):
                xs[pl.ds(b * Sq, 4 * Sq), :] = jnp.concatenate(
                    [x_buf[b + n].astype(f32) for n in range(4)], axis=0).astype(bf16)

        def clear():
            o_buf[...] = jnp.zeros_like(o_buf)
            acc[...] = jnp.zeros_like(acc)

        for i in range(LA):
            wq_half(0, i, 0, start[0])
        x_copy = pltpu.make_async_copy(x_hbm, x_buf, sem.at[0])
        x_copy.start()
        for i in range(LEAD):
            wq_half(0, i, 1, start[1])
            pl.delay(_DELAY_WQ)
        for i in range(LAG):
            wq_slot(0, i, (clear, None, prepare, None, None)[i])
        loop(LAG, NQ[0] - LA, lambda i: wq_slot(0, i))
        for i in range(NQ[0] - LA, NQ[0]):
            wq_slot(0, i)
        for i in range(LAG):
            wq_slot(1, i)
        loop(LAG, LAG + 4 * NJ, lambda i: wq_slot(1, i, lambda: project_q(0, i - LAG)))
        loop(LAG + 4 * NJ, NQ[1] - LA, lambda i: wq_slot(1, i))
        for i in range(NQ[1] - LA, NQ[1] + 2):
            wq_slot(1, i)

        def kv_step(t, first=False):
            for i in range(NS):
                kv_slot(t, i + LEAD, 1, start[1])
                if not first and i >= NS - 2:
                    pl.when(t + 1 == T)(lambda: start[1](wo_piece(0, 1, i - (NS - 2))))
                j = (i - LAG + 1) % NS
                if first and (j <= NS // 2 or j == NS - 1 or i < LAG - 1):
                    pl.delay(_DELAY_WQ)
                else:
                    pl.delay(_DELAY_KV[j])
                    if j <= NS // 2:
                        value(t - 1, j)
                    elif j < NS - 1:
                        score(t if i >= LAG - 1 else t - 1, j - NS // 2 - 1)
                    else:
                        n = (t & 31) - (32 - 4 * NJ)
                        lax.cond(jnp.logical_and(n >= 0, t < T - 32),
                                 lambda: project_q((t >> 5) + 1, n),
                                 lambda: pl.delay(_DELAY_IDLE))
                kv_slot(t, i + LA, 0, start[0])
                kv_slot(t, i, 0, wait)
                if first and i < LAG:
                    wq_half(1, NQ[1] + 2 + i - LAG, 1, wait)
                else:
                    kv_slot(t, i - LAG, 1, wait)
                if not first and NS - LA <= i < NS - LA + 2 * WA:
                    g, n = divmod(i - (NS - LA), 2)
                    pl.when(t + 1 == T)(lambda: start[0](wo_piece(g, 0, n)))

        kv_step(0, first=True)
        loop(1, T, kv_step)
        for i in range(LAG - 1):
            if i - LAG + 1 < -1:
                score(T - 1, NS // 2 + i - LAG)
        for i in range(LAG):
            kv_slot(T, i - LAG, 1, wait)

        def wait_high(g):
            wait(wo_piece(g, 1, 0))
            wait(wo_piece(g, 1, 1))

        def wo_group(g, work):
            for i in range(2):
                if i == 0:
                    pl.when(g > 0)(lambda: wait_high(g - 1))
                start[1](wo_piece(g + 1, 1, i))
                pl.delay(_DELAY_WO)
                work(i)
                pl.when(g + WA < NG)(lambda: start[0](wo_piece(g + WA, 0, i)))
                wait(wo_piece(g, 0, i))

        NF = 5
        for g in range(NF - 1):
            wo_group(g, lambda i: value(T - 1, 2 * g + i) if 2 * g + i <= 2 * NJ else None)

        def project(g):
            def work(i):
                n = 2 * (g - (NF - 1)) + i
                lax.cond(n < 2 * (NF - 2),
                         lambda: (project_o(2 * n), project_o(2 * n + 1), None)[-1],
                         lambda: project_o(2 * (g - 1) + i))
            return work

        loop(NF - 1, NG - 1, lambda g: wo_group(g, project(g)))
        wait_high(NG - 2)
        project_o(2 * NG - 4)
        project_o(2 * NG - 3)
        wait(wo_piece(NG - 1, 0, 0))
        wait_high(NG - 1)
        project_o(2 * NG - 1)
        wait(wo_piece(NG - 1, 0, 1))
        project_o(2 * NG - 2)
        for b in range(B):
            out_ref[b] = acc[pl.ds(b * Sq, Sq), :].astype(out_ref.dtype)

    kt = jnp.swapaxes(k_cache, 2, 3).reshape(B, HD, Sk)
    vt = jnp.swapaxes(v_cache, 2, 3).reshape(B, HD, Sk)

    any_spec = pl.BlockSpec(memory_space=pl.ANY)
    return pl.pallas_call(
        kernel,
        out_shape=jax.ShapeDtypeStruct((B, Sq, D), x.dtype),
        in_specs=[any_spec] * 5,
        out_specs=pl.BlockSpec(memory_space=pltpu.VMEM),
        scratch_shapes=[
            pltpu.VMEM((B, Sq, D), x.dtype),
            pltpu.VMEM((4, P, W), k_cache.dtype),
            pltpu.VMEM((4, P, W), v_cache.dtype),
            pltpu.VMEM(wq.shape, wq.dtype),
            pltpu.VMEM(wo.shape, wo.dtype),
            pltpu.VMEM((B * Sq, D), bf16),
            pltpu.VMEM((2, 4 * NJ, B * Sq, 128), f32),
            pltpu.VMEM((R, W), f32),
            pltpu.VMEM((R, W), bf16),
            pltpu.VMEM((R, P), f32),
            pltpu.VMEM((B * Sq, HD), f32),
            pltpu.VMEM((B * Sq, D), f32),
            pltpu.SemaphoreType.DMA((4,)),
        ],
        compiler_params=pltpu.CompilerParams(
            vmem_limit_bytes=64 * 1024 * 1024, disable_bounds_checks=_NOCHECK),
    )(x, kt, vt, wq, wo)
```

```python
import jax
import jax.numpy as jnp
from jax import lax
import jax.experimental.pallas as pl
import jax.experimental.pallas.tpu as pltpu

_SLOTS = 12
_FIRST = ((12, 37), (0, 17))
_AHEAD = (10, 1)
_LAG = 4
_WO_AHEAD = 3
_IDLE_HALF, _IDLE_WQ, _IDLE, _IDLE_NORM, _IDLE_SOFTMAX = 60, 115, 90, 65, 15


@jax.jit
def pallas_standalone__sliding_block_cached__sampling_kernel(
    x: jax.Array,
    k_cache: jax.Array,
    v_cache: jax.Array,
    wq: jax.Array,
    wo: jax.Array,
):
    B, Sq, D = x.shape
    Hq, Dh = 32, 192
    Hkv, Sk = k_cache.shape[1], k_cache.shape[2]
    W = min(4096, max(256, Sk // 4))
    assert Hq == Hkv and Sq == 4 and B == 8 and D % 64 == 0 and W % 256 == 0
    HD = Hq * Dh
    P = 2 * Dh
    NJ = P // 128
    R = 2 * Sq
    T = Hq // 2 * B
    NS, NK = _SLOTS, _SLOTS // 2
    NU = P // 32
    NB = max(_FIRST[0] + _FIRST[1]) // 8
    QW = 1024
    QB, QS = HD // QW, D // 64
    NG = HD // 256
    scale = Dh ** -0.5
    f32, bf16 = jnp.float32, jnp.bfloat16
    fragments = lambda rows, cols: (rows // 32, 2, 2, 8, cols)

    batch_of = lambda t: (t >> 2) & 7
    pair_of = lambda t: ((t >> 5) << 2) + (t & 3)

    def kernel(x_hbm, k_hbm, v_hbm, wq_hbm, wo_hbm, out_ref,
               x_buf, k_buf, v_buf, wq_buf, wo_buf, xs, q_buf, s_buf, p_buf, pv_buf,
               o_buf, acc, sem):
        start = (lambda c: c.start(priority=1), lambda c: c.start(priority=0))
        wait = lambda c: c.wait()
        both, one, two = slice(0, 2), slice(0, 1), slice(1, 2)

        def loop(lo, hi, body):
            lax.fori_loop(lo, hi, lambda i, c: (body(i), c)[1], 0)

        def kv_slot(t, i, hi, fn, pick=both):
            wrap, i = divmod(i, NS)
            which, blk = divmod(i, NK)
            src, buf = ((k_hbm, k_buf), (v_hbm, v_buf))[which]
            for first in _FIRST[hi][pick]:
                dt, f = divmod(8 * blk + first, 4 * NU)
                u = t + (wrap + dt)
                exists = 0 <= u < T if isinstance(u, int) else wrap + dt <= 0 or u < T

                @pl.when(exists)
                def _():
                    n = (batch_of(u) * (Hq // 2) + pair_of(u)) * NU + f // 4
                    fn(pltpu.make_async_copy(
                        src.at[n, :, f % 4, :, pl.ds(Sk - W, W)],
                        buf.at[u & 3, f // 4, :, f % 4], sem.at[2 * (u & 3) + which]))

        def wq_slot(i, hi, fn, pick=both):
            c, j = divmod(i, QS)
            for first in _FIRST[hi][pick]:
                dc, f = divmod(8 * j + first, 8 * QS)
                if 0 <= c + dc < QB:
                    part = (f // 4, both, f % 4, slice(None), pl.ds((c + dc) * QW, QW))
                    fn(pltpu.make_async_copy(
                        wq_hbm.at[part], wq_buf.at[part], sem.at[6 if c + dc < 2 else 7]))
            if i < 0:
                kv_slot(0, i, hi, fn, pick)
            elif i >= QB * QS:
                kv_slot(0, i - QB * QS, hi, fn, pick)
            elif i >= QB * QS - NB:
                kv_slot(0, i - QB * QS - NK, hi, fn, pick)

        def wo_piece(g, hi, i):
            rows = pl.ds(pl.multiple_of((hi * NG + g) * 128 + i * 64, 64), 64)
            return pltpu.make_async_copy(
                wo_hbm.at[rows], wo_buf.at[rows], sem.at[4 * hi + (g & 3)])

        def iota(shape, axis):
            return lax.broadcasted_iota(jnp.int32, shape, axis)

        def head_mask(shape, col0=0):
            return (iota(shape, 0) >= Sq) == (iota(shape, 1) + col0 >= Dh)

        def batch_mask(shape, b):
            return (iota(shape, 0) >> 2) == (b & 1)

        def batch_rows(b):
            return pl.ds(pl.multiple_of((b >> 1) * R, R), R)

        def project_q(g, n):
            cols = pl.ds(pl.multiple_of((g * 4 * NJ + n) * 128, 128), 128)
            w = wq_buf[:, :, :, :, cols].reshape(D, 128)
            q_buf[g & 1, n] = jnp.dot(xs[...], w, preferred_element_type=f32)

        def score(t, j):
            if j < NJ:
                b = batch_of(t)
                q = q_buf[(t >> 5) & 1, (t & 3) * NJ + j, batch_rows(b), :]
                q = jnp.where(batch_mask(q.shape, b), q, pltpu.roll(q, Sq, 0))
                q = jnp.where(head_mask(q.shape, j * 128), q, 0.0).astype(bf16)
                k = k_buf[t & 3, pl.ds(4 * j, 4)].reshape(128, W)
                d = jnp.dot(q, k, preferred_element_type=f32)
                s_buf[...] = d if j == 0 else s_buf[...] + d
            else:
                s = s_buf[...] * scale
                e = jnp.exp(s - jnp.max(s, axis=-1, keepdims=True))
                s_buf[...] = e
                p_buf[...] = e.astype(bf16)

        def value(t, j):
            if j < 2 * NJ:
                cols, keys = pl.ds(j // 2 * 128, 128), pl.ds(j % 2 * (W // 2), W // 2)
                v = v_buf[t & 3, pl.ds(j // 2 * 4, 4), :, :, :, keys].reshape(128, W // 2)
                d = lax.dot_general(p_buf[:, keys], v, (((1,), (1,)), ((), ())),
                                    preferred_element_type=f32)
                pv_buf[:, cols] = d if j % 2 == 0 else pv_buf[:, cols] + d
            else:
                b = batch_of(t)
                l = jnp.sum(s_buf[...], axis=-1, keepdims=True)
                o = jnp.where(head_mask((R, P)), pv_buf[...] / l, 0.0)
                o = o + pltpu.roll(o, Sq, 0)
                where = (batch_rows(b), pl.ds(pl.multiple_of(pair_of(t) * P, P), P))
                o_buf[where] = jnp.where(batch_mask((R, P), b), o, o_buf[where])

        def project_o(g, *queues):
            total = acc[...]
            for hi in queues:
                rows = pl.ds(pl.multiple_of((hi * NG + g) * 128, 128), 128)
                total += jnp.dot(o_buf[:, rows].astype(bf16), wo_buf[rows, :],
                                 preferred_element_type=f32)
            acc[...] = total

        def idle(ns, midway):
            pl.delay(_IDLE_HALF)
            midway()
            pl.delay(ns - _IDLE_HALF)

        def clear():
            o_buf[...] = jnp.zeros_like(o_buf)
            acc[...] = jnp.zeros_like(acc)

        def gather_x():
            x_copy.wait()
            for b in range(0, B, 4):
                xs[pl.ds(b * Sq, 4 * Sq), :] = jnp.concatenate(
                    [x_buf[b + n].astype(f32) for n in range(4)], axis=0).astype(bf16)

        for i in range(-NB, _AHEAD[0]):
            wq_slot(i, 0, start[0])
        x_copy = pltpu.make_async_copy(x_hbm, x_buf, sem.at[5])
        x_copy.start()
        for i in range(-NB, _AHEAD[1]):
            wq_slot(i, 1, start[1])
        for i in range(-NB, 0):
            wq_slot(i, 0, wait)
        for i in range(-NB, -_LAG):
            wq_slot(i, 1, wait)
        work = {0: clear, 1: gather_x}
        for n in range(4 * NJ):
            work[2 * QS + _LAG + n] = lambda n=n: project_q(0, n)
        for i in range(QB * QS):
            midway = lambda: wq_slot(i + _AHEAD[1], 1, start[1], two)
            wq_slot(i + _AHEAD[1], 1, start[1], one)
            if i in work:
                pl.delay(1)
                work[i]()
                midway()
            else:
                idle(_IDLE_WQ, midway)
            wq_slot(i + _AHEAD[0], 0, start[0])
            wq_slot(i, 0, wait)
            wq_slot(i - _LAG, 1, wait)

        def kv_step(t, first=False):
            for i in range(NS):
                midway = lambda: kv_slot(t, i + _AHEAD[1], 1, start[1], two)
                kv_slot(t, i + _AHEAD[1], 1, start[1], one)
                if not first and i >= NS - 2:
                    pl.when(t + 1 == T)(lambda: start[1](wo_piece(0, 1, i - (NS - 2))))
                j = (i - _LAG) % NS
                if first and i <= _LAG + NK:
                    idle(_IDLE, midway)
                elif j < NK:
                    pl.delay(1)
                    value(t - 1, j)
                    midway()
                elif j == NK:
                    idle(_IDLE_NORM, midway)
                    value(t - 1, j)
                elif j < NS - 1:
                    pl.delay(1 if j < NS - 2 else _IDLE_SOFTMAX)
                    score(t if i >= _LAG else t - 1, j - NK - 1)
                    midway()
                else:
                    n = (t & 31) - (32 - 4 * NJ)
                    lax.cond(jnp.logical_and(n >= 0, t < T - 32),
                             lambda: (project_q((t >> 5) + 1, n), midway(), None)[-1],
                             lambda: idle(_IDLE, midway))
                kv_slot(t, i + _AHEAD[0], 0, start[0])
                kv_slot(t, i, 0, wait)
                if first and i < _LAG:
                    wq_slot(QB * QS + i - _LAG, 1, wait)
                else:
                    kv_slot(t, i - _LAG, 1, wait)
                g, half = divmod(i + _AHEAD[0] - NS, 2)
                if not first and 0 <= g < _WO_AHEAD:
                    pl.when(t + 1 == T)(lambda: start[0](wo_piece(g, 0, half)))

        kv_step(0, first=True)
        loop(1, T, kv_step)
        for i in range(_LAG - 1):
            score(T - 1, NK - 1 + i - _LAG)
        for i in range(_LAG):
            kv_slot(T, i - _LAG, 1, wait)

        def wait_tile(g, hi):
            wait(wo_piece(g, hi, 0))
            wait(wo_piece(g, hi, 1))

        def wo_group(g, work):
            pl.when(g > 0)(lambda: wait_tile(g - 1, 1))
            for i in range(2):
                start[1](wo_piece(g + 1, 1, i))
                pl.delay(5)
                work(i)
                pl.when(g + _WO_AHEAD < NG)(
                    lambda: start[0](wo_piece(g + _WO_AHEAD, 0, i)))
                wait(wo_piece(g, 0, i))

        def project(g, i):
            n = 2 * (g - NF) + i
            lax.cond(n < 2 * (NF - 1),
                     lambda: project_o(n, 0, 1), lambda: project_o(g - 1, i))

        NF = NJ + 1
        for g in range(NF):
            wo_group(g, lambda i: value(T - 1, 2 * g + i) if 2 * g + i <= NK else None)
        loop(NF, NG - 1, lambda g: wo_group(g, lambda i: project(g, i)))
        wait_tile(NG - 2, 1)
        project_o(NG - 2, 0, 1)
        wait_tile(NG - 1, 1)
        wait_tile(NG - 1, 0)
        project_o(NG - 1, 0, 1)
        for b in range(B):
            out_ref[b] = acc[pl.ds(b * Sq, Sq), :].astype(out_ref.dtype)

    kt = jnp.swapaxes(k_cache, 2, 3).reshape(fragments(B * HD, Sk))
    vt = jnp.swapaxes(v_cache, 2, 3).reshape(fragments(B * HD, Sk))

    return pl.pallas_call(
        kernel,
        out_shape=jax.ShapeDtypeStruct((B, Sq, D), x.dtype),
        in_specs=[pl.BlockSpec(memory_space=pl.ANY)] * 5,
        out_specs=pl.BlockSpec(memory_space=pltpu.VMEM),
        scratch_shapes=[
            pltpu.VMEM((B, Sq, D), x.dtype),
            pltpu.VMEM((4,) + fragments(P, W), k_cache.dtype),
            pltpu.VMEM((4,) + fragments(P, W), v_cache.dtype),
            pltpu.VMEM(fragments(D, HD), wq.dtype),
            pltpu.VMEM(wo.shape, wo.dtype),
            pltpu.VMEM((B * Sq, D), bf16),
            pltpu.VMEM((2, 4 * NJ, B * Sq, 128), f32),
            pltpu.VMEM((R, W), f32),
            pltpu.VMEM((R, W), bf16),
            pltpu.VMEM((R, P), f32),
            pltpu.VMEM((B * Sq, HD), f32),
            pltpu.VMEM((B * Sq, D), f32),
            pltpu.SemaphoreType.DMA((8,)),
        ],
        compiler_params=pltpu.CompilerParams(vmem_limit_bytes=64 * 1024 * 1024),
    )(x, kt, vt, wq.reshape(fragments(D, HD)), wo)
```
